```python
import os as _os
_os.environ.setdefault("JAX_PLATFORMS", "cpu")
import jax
import jax.numpy as jnp

def _softmax(x, axis=-1):
    return jax.nn.softmax(x, axis=axis)
def _gelu(x):
    return jax.nn.gelu(x, approximate=True)
def _silu(x):
    return jax.nn.silu(x)
def _sigmoid(x):
    return jax.nn.sigmoid(x)
def _layernorm(x, axis=-1, eps=1e-5):
    m = jnp.mean(x, axis=axis, keepdims=True)
    v = jnp.var(x, axis=axis, keepdims=True)
    return (x - m) / jnp.sqrt(v + eps)
def _scatter_add(tgt, idx, src, axis=0):
    return tgt.at[idx].add(src)
def _segment_sum(src, seg, n):
    return jax.ops.segment_sum(src, seg, n)
class _Rng:
    def __init__(self, key):
        self._k = key
    def _next(self):
        self._k, sub = jax.random.split(self._k)
        return sub
    def normal(self, shape):
        return jax.random.normal(self._next(), shape, dtype=jnp.bfloat16)
    def randint(self, lo, hi, shape):
        return jax.random.randint(self._next(), shape, lo, hi, dtype=jnp.int32)
    def uniform(self, shape, lo=0.0, hi=1.0):
        return jax.random.uniform(self._next(), shape, jnp.bfloat16, lo, hi)
    def permutation(self, n):
        return jax.random.permutation(self._next(), n)


kernel_name = 'concat_heads__sliding_block__ssm_conv_s4__prompt'

def setup_inputs():
    _rng = _Rng(jax.random.key(int.from_bytes(__import__("os").urandom(4), "little")))
    _w = (lambda a: (lambda t: t.astype(jnp.bfloat16) if jnp.issubdtype(t.dtype, jnp.floating) else t)(jnp.asarray(a)))
    def _A_setup():
        B, S, D = 1, 2048, 512
        return {
            "x": _w((lambda *s: _rng.normal(s) * 0.2)(B, S, D)),
            "wqkv": _w((lambda *s: _rng.normal(s) * 0.2)(D, 3 * D)),
            "wo": _w((lambda *s: _rng.normal(s) * 0.05)(D, D)),
        }
    _A_in = _A_setup()

    def _B_setup():
        B, L, D, N = 1, 2048, 512, 128
        A_re = -jnp.exp((lambda *s: _rng.normal(s) * 0.8)(D, N))
        A_im = jnp.pi * (lambda *s: _rng.normal(s) * 0.8)(D, N)
        B_re = (lambda *s: _rng.normal(s) * 0.8)(D, N)
        B_im = (lambda *s: _rng.normal(s) * 0.8)(D, N)
        C_re = (lambda *s: _rng.normal(s) * 0.8)(D, N)
        C_im = (lambda *s: _rng.normal(s) * 0.8)(D, N)
        log_dt = (lambda *s: _rng.normal(s) * 0.8)(D) * 0.5 - 4.0
        Dskip = (lambda *s: _rng.normal(s) * 0.05)(D)
        return {
            "u": _w((lambda *s: _rng.normal(s) * 0.05)(B, L, D)),
            "A_re": _w(A_re),
            "A_im": _w(A_im),
            "B_re": _w(B_re),
            "B_im": _w(B_im),
            "C_re": _w(C_re),
            "C_im": _w(C_im),
            "log_dt": _w(log_dt),
            "Dskip": _w(Dskip),
        }
    _B_in = _B_setup()

    return {
        "A_x": _A_in["x"],
        "A_wqkv": _A_in["wqkv"],
        "A_wo": _A_in["wo"],
        "B_u": _B_in["u"],
        "B_A_re": _B_in["A_re"],
        "B_A_im": _B_in["A_im"],
        "B_B_re": _B_in["B_re"],
        "B_B_im": _B_in["B_im"],
        "B_C_re": _B_in["C_re"],
        "B_C_im": _B_in["C_im"],
        "B_log_dt": _B_in["log_dt"],
        "B_Dskip": _B_in["Dskip"],
    }

def reference(A_x, A_wqkv, A_wo, B_u, B_A_re, B_A_im, B_B_re, B_B_im, B_C_re, B_C_im, B_log_dt, B_Dskip):
    def _A_ref(x, wqkv, wo):
        B, S, D = x.shape
        H = 32; Dh = D // H; W = 256
        qkv = (lambda x, *d: x.transpose(*d))((x @ wqkv).reshape(B, S, 3, H, Dh), 2, 0, 3, 1, 4)
        q, k, v = qkv[0], qkv[1], qkv[2]
        scores = jnp.einsum("bhqd,bhkd->bhqk", q, k) * (Dh ** -0.5)
        idx = jnp.arange(S)
        mask = (idx[:, None] - idx[None, :] >= 0) & (idx[:, None] - idx[None, :] < W)
        scores = jnp.where(mask[None, None], scores, -1e9)
        p = _softmax(scores, axis=-1)
        o = jnp.einsum("bhqk,bhkd->bhqd", p, v)
        return (lambda x, *d: x.transpose(*d))(o, 0, 2, 1, 3).reshape(B, S, D) @ wo

    def _B_ref(u, A_re, A_im, B_re, B_im, C_re, C_im, log_dt, Dskip):
        Bsz, L, D = u.shape
        dt = jnp.exp(log_dt)[:, None]
        A = A_re + 1j * A_im
        Bc = B_re + 1j * B_im
        Cc = C_re + 1j * C_im
        logdA = dt * A
        dB = dt * Bc
        l = (lambda x, dt: x.astype(dt))(jnp.arange(L), A_re.dtype)
        P = jnp.exp(logdA[:, :, None] * l[None, None, :])
        K = jnp.einsum("dn,dnl,dn->dl", Cc, P, dB).real
        L2 = 2 * L
        Kp = jnp.pad(K, ((0, 0), (0, L)))
        up = (lambda x, *d: x.transpose(*d))(u, 0, 2, 1)
        up = jnp.pad(up, ((0, 0), (0, 0), (0, L)))
        Kf = (lambda x, axes=(-2,-1): jnp.fft.rfft2(x.astype(jnp.float32), axes=axes))(Kp[:, None, :], axes=(-2, -1))
        Uf = (lambda x, axes=(-2,-1): jnp.fft.rfft2(x.astype(jnp.float32), axes=axes))(up[:, :, None, :], axes=(-2, -1))
        Yf = Uf * Kf[None, :, :, :]
        y = (lambda x, s, axes=(-2,-1): jnp.fft.irfft2(x, s=s, axes=axes).astype(jnp.bfloat16))(Yf, (1, L2), axes=(-2, -1))[:, :, 0, :L]
        y = (lambda x, *d: x.transpose(*d))(y, 0, 2, 1) + u * Dskip[None, None, :]
        return y

    a = _A_ref(A_x, A_wqkv, A_wo)
    b = _B_ref(B_u, B_A_re, B_A_im, B_B_re, B_B_im, B_C_re, B_C_im, B_log_dt, B_Dskip)
    return jnp.concatenate([a, b], axis=-1)
```

```python
import math

import jax
import jax.numpy as jnp
import ml_dtypes
import numpy as np
from jax import lax
from jax.experimental import pallas as pl
from jax.experimental.pallas import tpu as pltpu

f32 = jnp.float32
bf16 = jnp.bfloat16
u32 = jnp.uint32
i32 = jnp.int32

S = 2048
D = 512
WIN = 256
T = 128
NCH = S // T
NMODE = 128

NT_DIMS = (((1,), (1,)), ((), ()))
TN_DIMS = (((0,), (0,)), ((), ()))

A_LIST = (1, 2, 3, 4, 5, 6, 7, 8, 258, 260, 262, 264, 516, 520, 772, 776, 1032, 1288, 1544, 1800)


def _idx_of(lp):
    if lp <= 256:
        return lp
    if lp <= 512:
        return 256 + (lp - 256) // 2
    if lp <= 1024:
        return 384 + (lp - 512) // 4
    return 512 + (lp - 1024) // 8


def _row_base_stride(a):
    base = _idx_of(a)
    return base, _idx_of(a + 8) - base


def _np_consts():
    bfn = ml_dtypes.bfloat16
    ks = np.concatenate([np.arange(0, T, 2), np.arange(1, T, 2)])
    s = np.arange(T)
    th = np.pi * (2.0 * ks[:, None] + 1.0) * s[None, :] / (2.0 * T)
    fc = np.cos(th) - 1j * np.sin(th)
    fmat = np.concatenate([fc.real, fc.imag], axis=0)
    gmat = np.concatenate([np.cos(th).T, -np.sin(th).T], axis=1) / T
    lr = np.arange(S).astype(bfn).astype(np.float64).astype(np.int64)
    fes = []
    for j in range(NCH):
        start = _idx_of(T * j)
        fe = np.zeros((T, T), np.complex128)
        for ss in range(T):
            lp = int(lr[T * j + ss])
            if lp == 0:
                continue
            fe[:, _idx_of(lp) - start] += fc[:, ss]
        fes.append(np.concatenate([fe.real, fe.imag], axis=0))
    groups = ((0,), (1,), (2, 3), (4, 5, 6, 7), tuple(range(8, 16)))
    for g in groups:
        for j in g[1:]:
            assert np.allclose(fes[j], fes[g[0]])
    fe5 = np.stack([fes[g[0]] for g in groups])
    ftype = [0] * NCH
    for ti, g in enumerate(groups):
        for j in g:
            ftype[j] = ti
    dft = np.concatenate([fmat[None], fe5], axis=0)
    lane = np.arange(128) // 16
    hm = np.stack([np.broadcast_to(np.where(lane == h, 0xFFFFFFFF, 0).astype(np.uint32), (32, 128))
                   for h in range(8)])
    return dft.astype(np.float32).astype(bfn), gmat.astype(np.float32).astype(bfn), np.ascontiguousarray(hm), tuple(ftype)


DFT_NP, G_NP, HM_NP, FTYPE = _np_consts()
KSTART = tuple(_idx_of(T * j) for j in range(NCH))
QSCALE = float(0.25 * math.log2(math.e))


def _bc(x, dt):
    return pltpu.bitcast(x, dt)


def _cmul(a, b):
    return a[0] * b[0] - a[1] * b[1], a[0] * b[1] + a[1] * b[0]


def _csq(a):
    return (a[0] + a[1]) * (a[0] - a[1]), (a[0] + a[0]) * a[1]


def _kernel(x_hbm, wqkv_hbm, wo_hbm, u_hbm, are_hbm, aim_hbm, bre_hbm, bim_hbm, cre_hbm, cim_hbm,
            ldt_hbm, dsk_hbm, dft_hbm, g_hbm, hm_hbm,
            out_hbm,
            x_v, w_v, wo_v, u_v, par_v, ldt_v, dsk_v, dft_v, g_v, hm_v,
            wvT_v, q_v, k_v, vt_v, ot_v, s0_v, s1_v,
            perm_v, wnat_v, coef_v, m_v, tr_v, kc_v, uh_v, kh_v, z_v,
            oa_v, ob_v, sems, osem):

    par_cp = [pltpu.make_async_copy(h, par_v.at[i], sems.at[i])
              for i, h in enumerate((are_hbm, aim_hbm, bre_hbm, bim_hbm, cre_hbm, cim_hbm))]
    ldt_cp = pltpu.make_async_copy(ldt_hbm, ldt_v, sems.at[6])
    dsk_cp = pltpu.make_async_copy(dsk_hbm, dsk_v, sems.at[7])
    w_cp = pltpu.make_async_copy(wqkv_hbm, w_v, sems.at[8])
    dft_cp = pltpu.make_async_copy(dft_hbm, dft_v, sems.at[9])
    g_cp = pltpu.make_async_copy(g_hbm, g_v, sems.at[10])
    hm_cp = pltpu.make_async_copy(hm_hbm, hm_v, sems.at[11])
    wo_cp = pltpu.make_async_copy(wo_hbm, wo_v, sems.at[12])
    x_cp = pltpu.make_async_copy(x_hbm.at[0], x_v, sems.at[13])
    u_cp = pltpu.make_async_copy(u_hbm.at[0], u_v, sems.at[14])

    def oa_cp(blk, slot):
        return pltpu.make_async_copy(oa_v.at[slot], out_hbm.at[0, pl.ds(blk * T, T), pl.ds(0, D)], osem.at[slot])

    def ob_cp(blk):
        return pltpu.make_async_copy(ob_v.at[pl.ds(blk * T, T), :], out_hbm.at[0, pl.ds(blk * T, T), pl.ds(D, D)],
                                     osem.at[2 + blk])

    for c in par_cp:
        c.start()
    ldt_cp.start()
    dsk_cp.start()
    w_cp.start()
    x_cp.start()
    dft_cp.start()
    u_cp.start()
    hm_cp.start()
    g_cp.start()
    wo_cp.start()

    k_v[0:WIN, :] = jnp.zeros((WIN, D), bf16)
    vt_v[:, 0:WIN] = jnp.zeros((D, WIN), bf16)
    kc_v[:, 0:8, :] = jnp.zeros((4, 8, 128), f32)
    kc_v[:, 640:768, :] = jnp.zeros((4, 128, 128), f32)

    for c in par_cp:
        c.wait()
    ldt_cp.wait()
    dsk_cp.wait()
    dt_row = jnp.exp(ldt_v[...].astype(f32)).astype(bf16).astype(f32).reshape(1, D)
    for sp in range(4):
        rows = slice(128 * sp, 128 * (sp + 1))
        dcol = jnp.broadcast_to(dt_row[:, rows], (128, 128)).T
        p = [par_v[i, rows, :].astype(f32) for i in range(6)]
        wr = (p[4] * p[2] - p[5] * p[3]) * dcol
        wi = (p[4] * p[3] + p[5] * p[2]) * dcol
        perm_v[0, pl.ds(sp, 128, stride=4), :] = p[0] * dcol
        perm_v[1, pl.ds(sp, 128, stride=4), :] = p[1] * dcol
        perm_v[2, pl.ds(sp, 128, stride=4), :] = wr
        perm_v[3, pl.ds(sp, 128, stride=4), :] = wi
        wnat_v[rows, :] = wr
    wn = wnat_v[...]
    whi = wn.astype(bf16)
    wlo = (wn - whi.astype(f32)).astype(bf16)
    ones = jnp.ones((16, 128), bf16)
    k0 = (lax.dot_general(ones, whi, NT_DIMS, preferred_element_type=f32)
          + lax.dot_general(ones, wlo, NT_DIMS, preferred_element_type=f32))
    coef_v[...] = k0[0:8] + dsk_v[...].astype(f32).reshape(1, D)

    w_cp.wait()
    wvT_v[...] = w_v[:, 2 * D:3 * D].T
    x_cp.wait()
    dft_cp.wait()
    u_cp.wait()

    sub8 = lax.broadcasted_iota(i32, (8, 128), 0)
    lane8 = lax.broadcasted_iota(i32, (8, 128), 1)

    def kgen(it):
        r0 = pl.multiple_of(it * 32, 32)
        zr = perm_v[0, pl.ds(r0, 32), :]
        zi = perm_v[1, pl.ds(r0, 32), :]
        w = (perm_v[2, pl.ds(r0, 32), :], perm_v[3, pl.ds(r0, 32), :])
        mag = jnp.exp(zr)
        L = {1: (mag * jnp.cos(zi), mag * jnp.sin(zi))}
        e = 1
        while e < 1024:
            L[2 * e] = _csq(L[e])
            e *= 2
        w256 = _cmul(w, L[256])
        w512 = _cmul(w, L[512])
        s0 = _cmul(_cmul(w, L[1024]), L[8])
        starts = [(_cmul(w, L[1]), _cmul(w, L[2])),
                  (_cmul(w256, L[2]), _cmul(w256, L[4])),
                  (_cmul(w512, L[4]), _cmul(w512, L[8])),
                  (s0, _cmul(s0, L[256]))]
        lo4 = sub8 < 4
        even = (lane8 & 1) == 0
        lt2 = (lane8 & 3) < 2
        acc = [None] * 20
        for h in range(4):
            rs = slice(8 * h, 8 * h + 8)

            def rep(z):
                zz = z[rs]
                zr_ = pltpu.roll(zz, 4, 0)
                return jnp.where(lo4, zz, zr_), jnp.where(lo4, zr_, zz)

            def mix(z0, z1):
                a0, a1 = z0[rs], z1[rs]
                return jnp.where(lo4, a0, pltpu.roll(a1, 4, 0)), jnp.where(lo4, pltpu.roll(a0, 4, 0), a1)

            def repc(z):
                r_, i_ = rep(z[0]), rep(z[1])
                return [(r_[0], i_[0]), (r_[1], i_[1])]

            def mixc(z0, z1):
                r_, i_ = mix(z0[0], z1[0]), mix(z0[1], z1[1])
                return [(r_[0], i_[0]), (r_[1], i_[1])]

            L2, L4, L256, L512 = repc(L[2]), repc(L[4]), repc(L[256]), repc(L[512])
            M = repc((L[16][0], -L[16][1]))
            one = jnp.ones((32, 128), f32)
            V0 = mixc((one, one - 1.0), (L[8][0], -L[8][1]))
            st = [mixc(s_[0], s_[1]) for s_ in starts]
            for gl in range(2):
                gi = 2 * h + gl
                t0 = st[0][gl]
                t1 = _cmul(t0, L2[gl])
                t2 = _cmul(t0, L4[gl])
                t3 = _cmul(t1, L4[gl])
                t4 = st[1][gl]
                t5 = _cmul(t4, L4[gl])
                t6 = st[2][gl]
                t7 = _cmul(t6, L256[gl])
                t8 = st[3][gl]
                t9 = _cmul(t8, L512[gl])
                ts = [t0, t1, t2, t3, t4, t5, t6, t7, t8, t9]
                vs = [V0[gl]]
                for _ in range(15):
                    vs.append(_cmul(vs[-1], M[gl]))
                tr = jnp.concatenate([t[0] for t in ts], axis=0).astype(bf16)
                ti = jnp.concatenate([t[1] for t in ts], axis=0).astype(bf16)
                vr = jnp.concatenate([v[0] for v in vs], axis=0).astype(bf16)
                vi = jnp.concatenate([v[1] for v in vs], axis=0).astype(bf16)
                o = (lax.dot_general(tr, vr, NT_DIMS, preferred_element_type=f32)
                     + lax.dot_general(ti, vi, NT_DIMS, preferred_element_type=f32))
                mg = sub8 == gi
                for i in range(10):
                    y = o[8 * i:8 * i + 8]
                    a_ = jnp.where(even, y, pltpu.roll(y, 7, 0))
                    b_ = jnp.where(lt2, a_, pltpu.roll(a_, 6, 0))
                    for xx in range(2):
                        sh = (gi - 4 * xx) % 8
                        v_ = b_ if sh == 0 else pltpu.roll(b_, sh, 0)
                        ai = 2 * i + xx
                        acc[ai] = v_ if gi == 0 else jnp.where(mg, v_, acc[ai])
        g0 = pl.multiple_of(it * 8, 8)
        for ai in range(20):
            m_v[ai, pl.ds(g0, 8), :] = acc[ai]

    def proj(it):
        r0 = pl.multiple_of(it * T, T)
        xb = x_v[pl.ds(r0, T), :]
        qk = jnp.dot(xb, w_v[:, 0:2 * D], preferred_element_type=f32)
        qh = pl.multiple_of(it * (T // 2), T // 2)
        q_v[pl.ds(qh, T // 2), :] = _bc((qk[:, 0:D] * QSCALE).astype(bf16), u32)
        k_v[pl.ds(r0 + WIN, T), :] = qk[:, D:2 * D].astype(bf16)
        vt = lax.dot_general(wvT_v[...], xb, NT_DIMS, preferred_element_type=f32)
        vt_v[:, pl.ds(r0 + WIN, T)] = vt.astype(bf16)

    def udft(it):
        r0 = pl.multiple_of(it * T, T)
        uh = jnp.dot(dft_v[0], u_v[pl.ds(r0, T), :], preferred_element_type=f32)
        for lt in range(4):
            a = uh[0:T, 128 * lt:128 * (lt + 1)]
            b = uh[T:2 * T, 128 * lt:128 * (lt + 1)]
            uh_v[0, it, lt] = a
            uh_v[1, it, lt] = b
            uh_v[2, it, lt] = a + b

    def p1(it, c):
        proj(it)
        kgen(it)
        udft(it)
        return c

    lax.fori_loop(0, NCH, p1, 0)

    for ai in range(20):
        tr_v[ai] = m_v[ai].T
    for ai, a in enumerate(A_LIST):
        base, stride = _row_base_stride(a)
        for sp in range(4):
            blk = tr_v[ai, pl.ds(sp, 32, stride=4), :]
            if stride == 1:
                kc_v[sp, base:base + 32, :] = blk
            else:
                kc_v[sp, pl.ds(base, 32, stride=stride), :] = blk
    for j in range(NCH):
        kw = jnp.concatenate([kc_v[sp, KSTART[j]:KSTART[j] + T, :] for sp in range(4)], axis=1).astype(bf16)
        kh = jnp.dot(dft_v[1 + FTYPE[j]], kw, preferred_element_type=f32)
        for lt in range(4):
            c_ = kh[0:T, 128 * lt:128 * (lt + 1)]
            d_ = kh[T:2 * T, 128 * lt:128 * (lt + 1)]
            kh_v[0, j, lt] = c_
            kh_v[1, j, lt] = d_ - c_
            kh_v[2, j, lt] = c_ + d_

    hm_cp.wait()
    wo_cp.wait()

    s_refs = (s0_v, s1_v)
    jj64 = lax.broadcasted_iota(i32, (64, 128), 0)
    ii64 = lax.broadcasted_iota(i32, (64, 128), 1) & 63
    NEG = -1e30

    def qk(Q0, j, t, s_ref, masked):
        q0 = Q0 + 64 * t
        cols = slice(128 * j, 128 * (j + 1))
        qb = q_v[pl.ds(pl.multiple_of(q0 // 2, 32), 32), cols]
        wT = _bc(jnp.concatenate([qb & hm_v[h] for h in range(8)], axis=0), bf16)
        kk = k_v[pl.ds(pl.multiple_of(q0, 64), 320), cols]
        sT = lax.dot_general(kk, wT, NT_DIMS, preferred_element_type=f32)
        farv = jnp.concatenate([jj64 > ii64] * 4, axis=1)
        far = sT[0:64]
        mid = sT[64:256]
        if masked:
            far = jnp.where(q0 - WIN + lax.broadcasted_iota(i32, (64, 512), 0) >= 0, far, NEG)
            mid = jnp.where(q0 - WIN + 64 + lax.broadcasted_iota(i32, (192, 512), 0) >= 0, mid, NEG)
        fold = jnp.where(farv, far, sT[256:320])
        s_ref[0:64, :] = fold
        s_ref[64:256, :] = mid
        return jnp.maximum(jnp.max(fold, axis=0, keepdims=True), jnp.max(mid, axis=0, keepdims=True))

    def smpv(Q0, j, t, s_ref, m):
        outs = []
        farv = jj64 > ii64
        zf = jnp.zeros((64, 128), f32)
        for pr in range(4):
            sl = slice(128 * pr, 128 * (pr + 1))
            p = jnp.exp2(s_ref[:, sl] - m[:, sl])
            l = jnp.sum(p, axis=0, keepdims=True)
            pf, pm = p[0:64], p[64:256]
            far = jnp.where(farv, pf, zf)
            near = jnp.where(farv, zf, pf)
            row = 128 * j + 32 * pr
            vA = vt_v[row:row + 32, pl.ds(Q0, 128)]
            vB = vt_v[row:row + 32, pl.ds(Q0 + 128, 128)]
            vC = vt_v[row:row + 32, pl.ds(Q0 + 256, 128)]
            cat = lambda a, b: jnp.concatenate([a, b], axis=0).astype(bf16)
            if t == 0:
                tA, tB, tC = cat(far, pm[0:64]), pm[64:192].astype(bf16), cat(near, zf)
            else:
                tA, tB, tC = cat(zf, far), pm[0:128].astype(bf16), cat(pm[128:192], near)
            o = (jnp.dot(vA, tA, preferred_element_type=f32) + jnp.dot(vB, tB, preferred_element_type=f32)
                 + jnp.dot(vC, tC, preferred_element_type=f32))
            outs.append(o * pl.reciprocal(l, approx=True))
        return outs

    lo64 = lax.broadcasted_iota(i32, (16, 128), 1) < 64

    def attn_block(Q0, Q0n, m, masked, masked_next):
        O = {}
        for n in range(8):
            j, t = n // 2, n % 2
            if n < 7:
                mn = qk(Q0, (n + 1) // 2, (n + 1) % 2, s_refs[(n + 1) % 2], masked)
            else:
                mn = qk(Q0n, 0, 0, s_refs[0], masked_next)
            O[t] = smpv(Q0, j, t, s_refs[n % 2], m)
            m = mn
            if t == 1:
                for pr in range(4):
                    o0, o1 = O[0][pr], O[1][pr]
                    zr_ = pltpu.roll(jnp.where(lo64, o1[0:16], o0[16:32]), 64, 1)
                    oh0 = jnp.where(lo64, o0[0:16], zr_)
                    oh1 = jnp.where(lo64, zr_, o1[16:32])
                    row = 128 * j + 32 * pr
                    ot_v[row:row + 32, :] = jnp.concatenate([oh0, oh1], axis=0)
        return m

    def outproj(blk):
        slot = blk % 2
        ot = ot_v[...].astype(bf16)
        o = lax.dot_general(ot, wo_v[...], TN_DIMS, preferred_element_type=f32)

        @pl.when(blk >= 2)
        def _():
            oa_cp(blk - 2, slot).wait()
        oa_v[slot] = o.astype(bf16)
        oa_cp(blk, slot).start()

    def mac(it):
        lt = it % 4
        for e in range(2):
            k0 = pl.multiple_of((it // 4) * 16 + 64 * e, 16)
            rows = pl.ds(k0, 16)
            zprev = None
            for m_ in range(NCH):
                t1 = t2 = t3 = None
                for c in range(m_ + 1):
                    jx = m_ - c
                    ua = uh_v[0, c, lt, rows, :]
                    ub = uh_v[1, c, lt, rows, :]
                    us = uh_v[2, c, lt, rows, :]
                    kc_ = kh_v[0, jx, lt, rows, :]
                    kdc = kh_v[1, jx, lt, rows, :]
                    kcd = kh_v[2, jx, lt, rows, :]
                    if t1 is None:
                        t1, t2, t3 = kc_ * us, ua * kdc, ub * kcd
                    else:
                        t1, t2, t3 = t1 + kc_ * us, t2 + ua * kdc, t3 + ub * kcd
                zre, zim = t1 - t3, t1 + t2
                if zprev is None:
                    ore, oim = zre, zim
                elif e == 0:
                    ore, oim = zre - zprev[1], zim + zprev[0]
                else:
                    ore, oim = zre + zprev[1], zim - zprev[0]
                zprev = (zre, zim)
                z_v[m_, lt, pl.ds(k0, 16), :] = ore
                z_v[m_, lt, pl.ds(pl.multiple_of(k0 + T, 16), 16), :] = oim

    def p2(it, m, masked, masked_next):
        Q0 = pl.multiple_of(it * T, T)
        Q0n = pl.multiple_of(jnp.minimum(it + 1, NCH - 1) * T, T)
        m = attn_block(Q0, Q0n, m, masked, masked_next)
        mac(it)
        outproj(it)
        return m

    m0 = qk(0, 0, 0, s0_v, True)
    m0 = lax.fori_loop(0, 2, lambda it, m: p2(it, m, True, True), m0)
    lax.fori_loop(2, NCH, lambda it, m: p2(it, m, False, False), m0)

    g_cp.wait()

    def p3(m_, c):
        r0 = pl.multiple_of(m_ * T, T)
        zz = jnp.concatenate([z_v[m_, lt] for lt in range(4)], axis=1).astype(bf16)
        y = jnp.dot(g_v[...], zz, preferred_element_type=f32)
        y = y + u_v[pl.ds(r0, T), :].astype(f32) * coef_v[0:1, :]
        ob_v[pl.ds(r0, T), :] = y.astype(bf16)
        ob_cp(m_).start()
        return c

    lax.fori_loop(0, NCH, p3, 0)
    oa_cp(NCH - 2, 0).wait()
    oa_cp(NCH - 1, 1).wait()
    for m_ in range(NCH):
        ob_cp(m_).wait()


@jax.jit
def pallas_concat_heads__sliding_block__ssm_conv_s4__prompt_kernel(
    A_x, A_wqkv, A_wo, B_u, B_A_re, B_A_im, B_B_re, B_B_im, B_C_re, B_C_im, B_log_dt, B_Dskip,
):
    anyspec = pl.BlockSpec(memory_space=pl.ANY)
    scratch = [
        pltpu.VMEM((S, D), bf16),
        pltpu.VMEM((D, 3 * D), bf16),
        pltpu.VMEM((D, D), bf16),
        pltpu.VMEM((S, D), bf16),
        pltpu.VMEM((6, D, NMODE), bf16),
        pltpu.VMEM((D,), bf16),
        pltpu.VMEM((D,), bf16),
        pltpu.VMEM((6, 2 * T, T), bf16),
        pltpu.VMEM((T, 2 * T), bf16),
        pltpu.VMEM((8, 32, 128), u32),
        pltpu.VMEM((D, D), bf16),
        pltpu.VMEM((S // 2, D), u32),
        pltpu.VMEM((S + WIN, D), bf16),
        pltpu.VMEM((D, S + WIN), bf16),
        pltpu.VMEM((D, T), f32),
        pltpu.VMEM((256, 512), f32),
        pltpu.VMEM((256, 512), f32),
        pltpu.VMEM((4, D, NMODE), f32),
        pltpu.VMEM((D, NMODE), f32),
        pltpu.VMEM((8, D), f32),
        pltpu.VMEM((20, 128, 128), f32),
        pltpu.VMEM((20, 128, 128), f32),
        pltpu.VMEM((4, 768, 128), f32),
        pltpu.VMEM((3, NCH, 4, T, 128), f32),
        pltpu.VMEM((3, NCH, 4, T, 128), f32),
        pltpu.VMEM((NCH, 4, 2 * T, 128), f32),
        pltpu.VMEM((2, T, D), bf16),
        pltpu.VMEM((S, D), bf16),
        pltpu.SemaphoreType.DMA((15,)),
        pltpu.SemaphoreType.DMA((2 + NCH,)),
    ]
    call = pl.pallas_call(
        _kernel,
        out_shape=jax.ShapeDtypeStruct((1, S, 2 * D), bf16),
        in_specs=[anyspec] * 15,
        out_specs=anyspec,
        scratch_shapes=scratch,
        compiler_params=pltpu.CompilerParams(vmem_limit_bytes=110 * 1024 * 1024),
    )
    return call(A_x, A_wqkv, A_wo, B_u, B_A_re, B_A_im, B_B_re, B_B_im, B_C_re, B_C_im, B_log_dt, B_Dskip,
                jnp.asarray(DFT_NP), jnp.asarray(G_NP), jnp.asarray(HM_NP))
```

```python
import math

import jax
import jax.numpy as jnp
import ml_dtypes
import numpy as np
from jax import lax
from jax.experimental import pallas as pl
from jax.experimental.pallas import tpu as pltpu

TOKPOS = (0, 11, 13, 15, 18)
OPOS = 2
OPN = 4
OPK = 1
XG = 4
PF = 2

f32 = jnp.float32
bf16 = jnp.bfloat16
u32 = jnp.uint32
i32 = jnp.int32

S = 2048
D = 512
WIN = 256
T = 128
NCH = S // T
NMODE = 128
UNR = 7
PRE = 2

NT_DIMS = (((1,), (1,)), ((), ()))
NEG = -1e30
QSCALE = float(0.25 * math.log2(math.e))

A_LIST = (1, 2, 3, 4, 5, 6, 7, 8, 258, 260, 262, 264, 516, 520, 772, 776, 1032, 1288, 1544, 1800)


def _idx_of(lp):
    if lp <= 256:
        return lp
    if lp <= 512:
        return 256 + (lp - 256) // 2
    if lp <= 1024:
        return 384 + (lp - 512) // 4
    return 512 + (lp - 1024) // 8


def _np_consts():
    bfn = ml_dtypes.bfloat16
    ks = np.concatenate([np.arange(0, T, 2), np.arange(1, T, 2)])
    s = np.arange(T)
    th = np.pi * (2.0 * ks[:, None] + 1.0) * s[None, :] / (2.0 * T)
    fc = np.cos(th) - 1j * np.sin(th)
    fmat = np.concatenate([fc.real, fc.imag], axis=0)
    gmat = np.concatenate([np.cos(th).T, -np.sin(th).T], axis=1) / T
    lr = np.arange(S).astype(bfn).astype(np.float64).astype(np.int64)
    fes = []
    for j in range(NCH):
        start = _idx_of(T * j)
        fe = np.zeros((T, T), np.complex128)
        for ss in range(T):
            lp = int(lr[T * j + ss])
            if lp != 0:
                fe[:, _idx_of(lp) - start] += fc[:, ss]
        fes.append(np.concatenate([fe.real, fe.imag], axis=0))
    groups = ((0,), (1,), (2, 3), (4, 5, 6, 7), tuple(range(8, 16)))
    ftype = [0] * NCH
    for ti, g in enumerate(groups):
        for j in g:
            assert np.allclose(fes[j], fes[g[0]])
            ftype[j] = ti
    dft = np.stack([fmat] + [fes[g[0]] for g in groups])
    order = np.concatenate([np.concatenate([np.arange(16 * b, 16 * b + 16), T + np.arange(16 * b, 16 * b + 16)])
                            for b in range(T // 16)])
    dft = dft[:, order, :]
    lane = np.arange(128) // 16
    hm = np.stack([np.broadcast_to(np.where(lane == h, 0xFFFFFFFF, 0).astype(np.uint32), (32, 128))
                   for h in range(8)])
    return (dft.astype(np.float32).astype(bfn), gmat.astype(np.float32).astype(bfn),
            np.ascontiguousarray(hm), tuple(ftype))


DFT_NP, G_NP, HM_NP, FTYPE = _np_consts()
KSTART = tuple(_idx_of(T * j) for j in range(NCH))
ALL_PASSES = tuple((kg, m0, p) for m0 in (12, 8, 4, 0) for kg in range(4) for p in range(3))


def _bc(x, dt):
    return pltpu.bitcast(x, dt)


def _mo(x, n):
    return x if isinstance(x, int) else pl.multiple_of(x, n)


def _cmul(a, b):
    return a[0] * b[0] - a[1] * b[1], a[0] * b[1] + a[1] * b[0]


def _csq(a):
    return (a[0] + a[1]) * (a[0] - a[1]), (a[0] + a[0]) * a[1]


def _kernel(x_hbm, wqkv_hbm, wo_hbm, u_hbm, are_hbm, aim_hbm, bre_hbm, bim_hbm, cre_hbm, cim_hbm,
            ldt_hbm, dsk_hbm, dft_hbm, g_hbm, hm_hbm,
            out_hbm,
            x_v, w_v, wo_v, u_v, par_v, ldt_v, dsk_v, dft_v, g_v, hm_v,
            wvT_v, wqk_v, woT_v, f_v, fe_v, gp_v, q_v, k_v, vt_v, ot_v, s0_v, s1_v,
            perm_v, wnat_v, coef_v, raw_v, m_v, tr_v, kc_v, uh_v, kh_v, z_v,
            oa_v, ob_v, sems, osem, xsem):

    par_cp = [pltpu.make_async_copy(h, par_v.at[i], sems.at[10 + i])
              for i, h in enumerate((are_hbm, aim_hbm, bre_hbm, bim_hbm, cre_hbm, cim_hbm))]
    ldt_cp = pltpu.make_async_copy(ldt_hbm, ldt_v, sems.at[0])
    dsk_cp = pltpu.make_async_copy(dsk_hbm, dsk_v, sems.at[1])
    w_cp = [pltpu.make_async_copy(wqkv_hbm.at[:, pl.ds(i * D, D)], w_v.at[:, pl.ds(i * D, D)], sems.at[2 + i])
            for i in range(3)]
    f_cp = pltpu.make_async_copy(dft_hbm.at[0], dft_v.at[0], sems.at[5])
    fe_cp = pltpu.make_async_copy(dft_hbm.at[pl.ds(1, 5)], dft_v.at[pl.ds(1, 5)], sems.at[6])
    g_cp = pltpu.make_async_copy(g_hbm, g_v, sems.at[7])
    hm_cp = pltpu.make_async_copy(hm_hbm, hm_v, sems.at[8])
    wo_cp = pltpu.make_async_copy(wo_hbm, wo_v, sems.at[9])

    def x_cp(i):
        return pltpu.make_async_copy(x_hbm.at[0, pl.ds(i * T, T), :], x_v.at[pl.ds(i * T, T), :], xsem.at[i])

    def u_cp(i):
        return pltpu.make_async_copy(u_hbm.at[0, pl.ds(i * T, T), :], u_v.at[pl.ds(i * T, T), :],
                                     xsem.at[NCH + i])

    def oa_cp(blk):
        return pltpu.make_async_copy(oa_v.at[pl.ds(blk * T, T), :], out_hbm.at[0, pl.ds(blk * T, T), pl.ds(0, D)],
                                     osem.at[NCH + blk])

    def ob_cp(blk):
        return pltpu.make_async_copy(ob_v.at[pl.ds(blk * T, T), :], out_hbm.at[0, pl.ds(blk * T, T), pl.ds(D, D)],
                                     osem.at[blk])

    for c in par_cp:
        c.start()
    ldt_cp.start()
    dsk_cp.start()
    w_cp[0].start()
    x_cp(0).start()
    x_cp(1).start()
    w_cp[2].start()
    f_cp.start()
    u_cp(0).start()
    u_cp(1).start()
    w_cp[1].start()

    kc_v[:, 0:8, :] = jnp.zeros((4, 8, 128), f32)
    kc_v[:, 640:768, :] = jnp.zeros((4, 128, 128), f32)
    z_v[0] = jnp.zeros((4, 3 * T, 128), f32)
    z_v[NCH + 1, 0, 0:8, :] = jnp.zeros((8, 128), f32)
    oa_v[S:S + 16, 0:128] = jnp.zeros((16, 128), bf16)

    for c in par_cp:
        c.wait()
    ldt_cp.wait()
    dsk_cp.wait()
    for i in range(2, 2 * PF):
        x_cp(i).start()
        u_cp(i).start()
    dt_row = jnp.exp(ldt_v[...].astype(f32)).astype(bf16).astype(f32).reshape(1, D)
    for sp in range(4):
        rows = slice(128 * sp, 128 * (sp + 1))
        dcol = jnp.broadcast_to(dt_row[:, rows], (128, 128)).T
        p = [par_v[i, rows, :].astype(f32) for i in range(6)]
        wr = (p[4] * p[2] - p[5] * p[3]) * dcol
        wi = (p[4] * p[3] + p[5] * p[2]) * dcol
        perm_v[0, pl.ds(sp, 128, stride=4), :] = p[0] * dcol
        perm_v[1, pl.ds(sp, 128, stride=4), :] = p[1] * dcol
        perm_v[2, pl.ds(sp, 128, stride=4), :] = wr
        perm_v[3, pl.ds(sp, 128, stride=4), :] = wi
        wnat_v[rows, :] = wr
    wn = wnat_v[...]
    whi = wn.astype(bf16)
    wlo = (wn - whi.astype(f32)).astype(bf16)
    ones = jnp.ones((16, 128), bf16)
    k0 = (lax.dot_general(ones, whi, NT_DIMS, preferred_element_type=f32)
          + lax.dot_general(ones, wlo, NT_DIMS, preferred_element_type=f32))
    coef_v[...] = k0[0:8] + dsk_v[...].astype(f32).reshape(1, D)

    sub8 = lax.broadcasted_iota(i32, (8, 128), 0)
    lane8 = lax.broadcasted_iota(i32, (8, 128), 1)
    lo4 = sub8 < 4

    def kgen_base(it):
        r0 = _mo(it * 32, 32)
        zr = perm_v[0, pl.ds(r0, 32), :]
        zi = perm_v[1, pl.ds(r0, 32), :]
        w = (perm_v[2, pl.ds(r0, 32), :], perm_v[3, pl.ds(r0, 32), :])
        mag = jnp.exp(zr)
        L = {1: (mag * jnp.cos(zi), mag * jnp.sin(zi))}
        e = 1
        while e < 1024:
            L[2 * e] = _csq(L[e])
            e *= 2
        w256 = _cmul(w, L[256])
        w512 = _cmul(w, L[512])
        s0 = _cmul(_cmul(w, L[1024]), L[8])
        starts = [(_cmul(w, L[1]), _cmul(w, L[2])),
                  (_cmul(w256, L[2]), _cmul(w256, L[4])),
                  (_cmul(w512, L[4]), _cmul(w512, L[8])),
                  (s0, _cmul(s0, L[256]))]
        return L, starts

    def kgen_pair(base, h, slot):
        L, starts = base
        rs = slice(8 * h, 8 * h + 8)

        def rep(z):
            zz = z[rs]
            zr_ = pltpu.roll(zz, 4, 0)
            return jnp.where(lo4, zz, zr_), jnp.where(lo4, zr_, zz)

        def mix(z0, z1):
            a0, a1 = z0[rs], z1[rs]
            return jnp.where(lo4, a0, pltpu.roll(a1, 4, 0)), jnp.where(lo4, pltpu.roll(a0, 4, 0), a1)

        def repc(z):
            r_, i_ = rep(z[0]), rep(z[1])
            return [(r_[0], i_[0]), (r_[1], i_[1])]

        def mixc(z0, z1):
            r_, i_ = mix(z0[0], z1[0]), mix(z0[1], z1[1])
            return [(r_[0], i_[0]), (r_[1], i_[1])]

        L2, L4, L256, L512 = repc(L[2]), repc(L[4]), repc(L[256]), repc(L[512])
        M = repc((L[16][0], -L[16][1]))
        one = jnp.ones((32, 128), f32)
        V0 = mixc((one, one - 1.0), (L[8][0], -L[8][1]))
        st = [mixc(s_[0], s_[1]) for s_ in starts]
        for gl in range(2):
            t0 = st[0][gl]
            t1 = _cmul(t0, L2[gl])
            t2 = _cmul(t0, L4[gl])
            t3 = _cmul(t1, L4[gl])
            t4 = st[1][gl]
            t5 = _cmul(t4, L4[gl])
            t6 = st[2][gl]
            t7 = _cmul(t6, L256[gl])
            t8 = st[3][gl]
            t9 = _cmul(t8, L512[gl])
            ts = [t0, t1, t2, t3, t4, t5, t6, t7, t8, t9]
            vs = [V0[gl]]
            for _ in range(15):
                vs.append(_cmul(vs[-1], M[gl]))
            tr = jnp.concatenate([t[0] for t in ts], axis=0).astype(bf16)
            ti = jnp.concatenate([t[1] for t in ts], axis=0).astype(bf16)
            vr = jnp.concatenate([v[0] for v in vs], axis=0).astype(bf16)
            vi = jnp.concatenate([v[1] for v in vs], axis=0).astype(bf16)
            raw_v[slot, 2 * h + gl] = (lax.dot_general(tr, vr, NT_DIMS, preferred_element_type=f32)
                                       + lax.dot_general(ti, vi, NT_DIMS, preferred_element_type=f32))

    def kgen_extract(it, slot):
        even = (lane8 & 1) == 0
        lt2 = (lane8 & 3) < 2
        g0 = _mo(it * 8, 8)
        for i in range(10):
            acc = [None, None]
            for gi in range(8):
                y = raw_v[slot, gi, 8 * i:8 * i + 8, :]
                a_ = jnp.where(even, y, pltpu.roll(y, 7, 0))
                b_ = jnp.where(lt2, a_, pltpu.roll(a_, 6, 0))
                mg = sub8 == gi
                for xx in range(2):
                    sh = (gi - 4 * xx) % 8
                    v_ = b_ if sh == 0 else pltpu.roll(b_, sh, 0)
                    acc[xx] = v_ if gi == 0 else jnp.where(mg, v_, acc[xx])
            m_v[2 * i, pl.ds(g0, 8), :] = acc[0]
            m_v[2 * i + 1, pl.ds(g0, 8), :] = acc[1]

    def proj_q(it):
        q = jnp.dot(x_v[pl.ds(_mo(it * T, T), T), :], _bc(wqk_v[:, 0:D], bf16), preferred_element_type=f32)
        q_v[pl.ds(_mo(it * 64, 64), 64), :] = _bc((q * QSCALE).astype(bf16), u32)

    def proj_k(it):
        k = jnp.dot(x_v[pl.ds(_mo(it * T, T), T), :], _bc(wqk_v[:, D:2 * D], bf16), preferred_element_type=f32)
        k_v[pl.ds(_mo(it * 64, 64), 64), :] = _bc(k.astype(bf16), u32)

    def proj_vt(it):
        r0 = _mo(it * T, T)
        vt = lax.dot_general(_bc(wvT_v[...], bf16), x_v[pl.ds(r0, T), :], NT_DIMS, preferred_element_type=f32)
        vt_v[:, pl.ds(r0, T)] = _bc(vt.astype(bf16), u32)

    def dft_u(it):
        uh = jnp.dot(_bc(f_v[...], bf16), u_v[pl.ds(_mo(it * T, T), T), :], preferred_element_type=f32)
        for bb in range(T // 16):
            for lt in range(4):
                a = uh[32 * bb:32 * bb + 16, 128 * lt:128 * (lt + 1)]
                b = uh[32 * bb + 16:32 * bb + 32, 128 * lt:128 * (lt + 1)]
                uh_v[0, it, lt, 16 * bb:16 * bb + 16, :] = a
                uh_v[1, it, lt, 16 * bb:16 * bb + 16, :] = b
                uh_v[2, it, lt, 16 * bb:16 * bb + 16, :] = a + b

    def octet(base, o):
        kgen_pair(base, 0, o)
        kgen_pair(base, 1, o)
        kgen_pair(base, 2, o)
        kgen_pair(base, 3, o)
        kgen_extract(o, o)

    octet(kgen_base(0), 0)
    w_cp[0].wait()
    x_cp(0).wait()
    x_cp(1).wait()
    wqk_v[:, 0:D] = _bc(w_v[:, 0:D], u32)
    b1 = kgen_base(1)
    proj_q(0)
    kgen_pair(b1, 0, 1)
    kgen_pair(b1, 1, 1)
    proj_q(1)
    w_cp[2].wait()
    wvT_v[...] = _bc(w_v[:, 2 * D:3 * D].T, u32)
    kgen_pair(b1, 2, 1)
    kgen_pair(b1, 3, 1)
    kgen_extract(1, 1)
    b2 = kgen_base(2)
    proj_vt(0)
    kgen_pair(b2, 0, 2)
    proj_vt(1)
    f_cp.wait()
    u_cp(0).wait()
    u_cp(1).wait()
    f_v[...] = _bc(dft_v[0], u32)
    w_cp[1].wait()
    wqk_v[:, D:2 * D] = _bc(w_v[:, D:2 * D], u32)
    kgen_pair(b2, 1, 2)
    kgen_pair(b2, 2, 2)
    kgen_pair(b2, 3, 2)
    kgen_extract(2, 2)
    b3 = kgen_base(3)
    dft_u(0)
    kgen_pair(b3, 0, 3)
    dft_u(1)
    kgen_pair(b3, 1, 3)
    proj_k(0)
    kgen_pair(b3, 2, 3)
    kgen_pair(b3, 3, 3)
    proj_k(1)
    kgen_extract(3, 3)
    for e in range(2):
        x_cp(2 * PF + e).start()
        u_cp(2 * PF + e).start()

    def p1(i, with_kg):
        for e in range(2):
            x_cp(2 * i + e).wait()
            u_cp(2 * i + e).wait()

        @pl.when(i + PF < NCH // 2)
        def _():
            for e in range(2):
                x_cp(2 * (i + PF) + e).start()
                u_cp(2 * (i + PF) + e).start()

        if with_kg:
            @pl.when(i == 1)
            def _():
                fe_cp.start()
                hm_cp.start()
                wo_cp.start()
                g_cp.start()

        for e in range(2):
            it = 2 * i + e
            if with_kg:
                base = kgen_base(it + PRE)
            for h, step in enumerate((proj_q, dft_u, proj_vt, proj_k)):
                step(it)
                if with_kg:
                    kgen_pair(base, h, e)
            if with_kg:
                kgen_extract(it + PRE, e)
        return i

    n_kg = (NCH - PRE) // 2
    last = lax.fori_loop(1, n_kg, lambda i, c: p1(i, True), 0)
    lax.fori_loop(n_kg, NCH // 2, lambda i, c: p1(i, False), 0)
    zd = last - (n_kg - 1)

    for ai in range(20):
        tr_v[ai] = m_v[ai].T
    for ai, a in enumerate(A_LIST):
        base = _idx_of(a)
        stride = _idx_of(a + 8) - base
        for sp in range(4):
            blk = tr_v[ai, pl.ds(sp, 32, stride=4), :]
            if stride == 1:
                kc_v[sp, base:base + 32, :] = blk
            else:
                kc_v[sp, pl.ds(base, 32, stride=stride), :] = blk
    fe_cp.wait()
    for ti in range(5):
        fe_v[ti] = _bc(dft_v[1 + ti], u32)
    hm_cp.wait()
    wo_cp.wait()
    woT_v[...] = _bc(wo_v[...].T, u32)

    def dft_k(j):
        kw = jnp.concatenate([kc_v[sp, KSTART[j]:KSTART[j] + T, :] for sp in range(4)], axis=1)
        kh = jnp.dot(_bc(fe_v[FTYPE[j]], bf16), kw.astype(bf16), preferred_element_type=f32)
        for bb in range(T // 16):
            for lt in range(4):
                c_ = kh[32 * bb:32 * bb + 16, 128 * lt:128 * (lt + 1)]
                d_ = kh[32 * bb + 16:32 * bb + 32, 128 * lt:128 * (lt + 1)]
                kh_v[0, j, lt, 16 * bb:16 * bb + 16, :] = c_
                kh_v[1, j, lt, 16 * bb:16 * bb + 16, :] = d_ - c_
                kh_v[2, j, lt, 16 * bb:16 * bb + 16, :] = c_ + d_

    def mac_pass(it, kg, m0, p):
        lt = it % 4
        ltd = lt + zd if isinstance(it, int) else lt
        k0 = _mo((it // 4) * 32 + 8 * kg, 8)
        rows = pl.ds(k0, 8)
        kp, up = ((0, 2), (1, 0), (2, 1))[p]
        kw = {}
        acc = [None] * 4
        for c in range(m0 + 4):
            uu = uh_v[up, c, lt, rows, :]
            for i in range(4):
                jx = m0 + i - c
                if jx < 0:
                    continue
                if jx not in kw:
                    kw[jx] = kh_v[kp, jx, lt, rows, :]
                pr_ = kw[jx] * uu
                acc[i] = pr_ if acc[i] is None else acc[i] + pr_
        for i in range(4):
            z_v[m0 + i + 1, ltd, pl.ds(_mo(k0 + p * T, 8), 8), :] = acc[i]

    def slot_groups(it, n):
        kg = n // 2
        if n % 2 == 0:
            g = [[(kg, 12, 0)], [(kg, 12, 1)], [(kg, 12, 2)], [(kg, 4, 0)], [(kg, 0, 0), (kg, 0, 1), (kg, 0, 2)]]
        else:
            g = [[(kg, 8, 0)], [(kg, 8, 1)], [(kg, 8, 2)], [(kg, 4, 1)], [(kg, 4, 2)]]
        return [[(it,) + e for e in grp] for grp in g]

    s_refs = (s0_v, s1_v)
    jj64 = lax.broadcasted_iota(i32, (64, 128), 0)
    ii64 = lax.broadcasted_iota(i32, (64, 128), 1) & 63
    farv = jj64 > ii64

    def qk(q0, j, s_ref, groups=None, tko=None):
        head = isinstance(q0, int) and q0 < WIN
        cols = slice(128 * j, 128 * (j + 1))
        qa = _mo(q0 // 2, 32)
        qb = q_v[pl.ds(qa, 32), cols]
        wT = _bc(jnp.concatenate([qb & hm_v[h] for h in range(8)], axis=0), bf16)
        parts = []
        if head:
            nm = q0
            for i in range(4):
                parts.append(k_v[pl.ds(qa + 8 * i, 8), cols])
            for i in range(nm // 16):
                parts.append(k_v[8 * i:8 * i + 8, cols])
        else:
            nm = 192
            for i in range(4):
                parts.append(k_v[pl.ds(qa - WIN // 2 + 8 * i, 8), cols])
                parts.append(k_v[pl.ds(qa + 8 * i, 8), cols])
            for i in range(12):
                parts.append(k_v[pl.ds(qa - 96 + 8 * i, 8), cols])
        if tko is not None:
            parts[OPK] = parts[OPK] | tko
        if groups is not None:
            for gi, grp in enumerate(groups):
                for (it_, kg, m0, p) in grp:
                    mac_pass(it_, kg, m0, p)
                parts[TOKPOS[gi]] = parts[TOKPOS[gi]] | _bc(z_v[NCH + 1, 0, 0:8, :], u32)
        sT = lax.dot_general(_bc(jnp.concatenate(parts, axis=0), bf16), wT, NT_DIMS,
                             preferred_element_type=f32)
        if head:
            near, mid = sT[0:64], (sT[64:64 + nm] if nm else None)
            far = jnp.full((64, 512), NEG, f32)
        else:
            far = jnp.concatenate([sT[32 * i:32 * i + 16] for i in range(4)], axis=0)
            near = jnp.concatenate([sT[32 * i + 16:32 * i + 32] for i in range(4)], axis=0)
            mid = sT[128:320]
        fold = jnp.where(jnp.concatenate([farv] * 4, axis=1), far, near)
        mx = jnp.max(fold, axis=0, keepdims=True)
        for pr in range(4):
            s_ref[pr, 0:64, :] = fold[:, 128 * pr:128 * (pr + 1)]
            if nm:
                s_ref[pr, 64:64 + nm, :] = mid[:, 128 * pr:128 * (pr + 1)]
        if nm:
            mx = jnp.maximum(mx, jnp.max(mid, axis=0, keepdims=True))
        return mx

    def sm(Q0, t, s_ref, m):
        head = isinstance(Q0, int) and Q0 < WIN
        nm = Q0 + 64 * t if head else 192
        zf = jnp.zeros((64, 128), f32)
        cat = lambda a, b: jnp.concatenate([a, b], axis=0).astype(bf16)
        res = []
        for pr in range(4):
            p = jnp.exp2(s_ref[pr, 0:64 + nm, :] - m[:, 128 * pr:128 * (pr + 1)])
            acc = None
            for c in range(0, 64 + nm, 32):
                r = (p[c:c + 8] + p[c + 8:c + 16] + p[c + 16:c + 24]) + p[c + 24:c + 32]
                acc = r if acc is None else acc + r
            l = jnp.sum(acc, axis=0, keepdims=True)
            pf, pm = p[0:64], (p[64:64 + nm] if nm else None)
            if head:
                if t == 0:
                    tiles = ([(1, pm.astype(bf16))] if nm else []) + [(2, cat(pf, zf))]
                else:
                    tiles = ([(1, pm[0:128].astype(bf16))] if nm == 192 else []) + [(2, cat(pm[nm - 64:nm], pf))]
            else:
                far = jnp.where(farv, pf, zf)
                near = jnp.where(farv, zf, pf)
                if t == 0:
                    tiles = [(0, cat(far, pm[0:64])), (2, cat(near, zf)), (1, pm[64:192].astype(bf16))]
                else:
                    tiles = [(0, cat(zf, far)), (2, cat(pm[128:192], near)), (1, pm[0:128].astype(bf16))]
            res.append((tiles, l))
        return res

    def pv(Q0, j, t, res, slot):
        for pr in range(4):
            tiles, l = res[pr]
            row = 64 * j + 16 * pr
            o = None
            for ti, pt in tiles:
                v = vt_v[row:row + 16, pl.ds(Q0 + 128 * (ti - 2), 128)]
                d = jnp.dot(_bc(v, bf16), pt, preferred_element_type=f32)
                o = d if o is None else o + d
            o = o * pl.reciprocal(l, approx=False)
            r2 = 2 * row
            if t == 0:
                ot_v[slot, r2:r2 + 16, 0:64] = o[0:16, 0:64]
                ot_v[slot, r2 + 16:r2 + 32, 0:64] = pltpu.roll(o[16:32], 64, 1)[:, 0:64]
            else:
                ot_v[slot, r2:r2 + 16, 64:128] = pltpu.roll(o[0:16], 64, 1)[:, 64:128]
                ot_v[slot, r2 + 16:r2 + 32, 64:128] = o[16:32, 64:128]

    def outproj(blk, slot):
        oT = jnp.dot(_bc(woT_v[...], bf16), ot_v[slot].astype(bf16), preferred_element_type=f32)
        oa_v[pl.ds(_mo(blk * T, T), T), :] = oT.T.astype(bf16)
        return _bc(oa_v[S:S + 16, 0:128].astype(f32)[0:8], u32)

    def block(it, m, Q0, Q0n, slot, macs=None, extra=None):
        tko = None
        for n in range(8):
            j, t = n // 2, n % 2
            res = sm(Q0, t, s_refs[n % 2], m)
            g = macs(n) if macs is not None else None
            if n < 7:
                mn = qk(Q0 + 64 * ((n + 1) % 2), (n + 1) // 2, s_refs[(n + 1) % 2], g, tko if n == OPN else None)
                if n == OPOS and not (isinstance(it, int) and it == 0):
                    tko = outproj(it - 1, (slot - 1) % UNR)
            else:
                mn = qk(Q0n, 0, s_refs[0], g)
            if extra is not None:
                extra(n)
            pv(Q0, j, t, res, slot)
            m = mn
        return m

    m0 = qk(0, 0, s0_v)
    m0 = block(0, m0, 0, T, UNR - 2, None, lambda n: dft_k(n))
    m0 = block(1, m0, T, 2 * T, UNR - 1, None, lambda n: dft_k(8 + n))
    oa_cp(0).start()

    def p2(i, m):
        for e in range(UNR):
            it = 2 + i * UNR + e

            def macs(n, it=it, e=e):
                g = slot_groups(it, n)
                ex = ALL_PASSES[e::UNR]
                if n < len(ex):
                    g[XG] = g[XG] + [(i,) + ex[n]]
                return g
            m = block(it, m, _mo(it * T, T), _mo(jnp.minimum(it + 1, NCH - 1) * T, T), e, macs)
            oa_cp(it - 1).start()
        return m

    lax.fori_loop(0, (NCH - 2) // UNR, p2, m0)

    g_cp.wait()
    gp_v[...] = _bc(g_v[...], u32)

    def zplanes(mm):
        tt = jnp.concatenate([z_v[mm, lt] for lt in range(4)], axis=1)
        return tt[0:T] - tt[2 * T:3 * T], tt[0:T] + tt[T:2 * T]

    for m_ in range(NCH):
        zre, zim = zplanes(m_ + 1)
        pre, pim = zplanes(m_)
        zz = jnp.concatenate([zre[0:64] - pim[0:64], zre[64:128] + pim[64:128],
                              zim[0:64] + pre[0:64], zim[64:128] - pre[64:128]], axis=0).astype(bf16)
        y = jnp.dot(_bc(gp_v[...], bf16), zz, preferred_element_type=f32)
        y = y + u_v[m_ * T:(m_ + 1) * T, :].astype(f32) * coef_v[0:1, :]
        ob_v[m_ * T:(m_ + 1) * T, :] = y.astype(bf16)
        ob_cp(m_).start()
        if m_ == NCH // 2:
            outproj(NCH - 1, UNR - 1)
            oa_cp(NCH - 1).start()

    for m_ in range(NCH):
        oa_cp(m_).wait()
        ob_cp(m_).wait()


@jax.jit
def pallas_concat_heads__sliding_block__ssm_conv_s4__prompt_kernel(
    A_x: jax.Array,
    A_wqkv: jax.Array,
    A_wo: jax.Array,
    B_u: jax.Array,
    B_A_re: jax.Array,
    B_A_im: jax.Array,
    B_B_re: jax.Array,
    B_B_im: jax.Array,
    B_C_re: jax.Array,
    B_C_im: jax.Array,
    B_log_dt: jax.Array,
    B_Dskip: jax.Array,
):
    anyspec = pl.BlockSpec(memory_space=pl.ANY)
    scratch = [
        pltpu.VMEM((S, D), bf16),
        pltpu.VMEM((D, 3 * D), bf16),
        pltpu.VMEM((D, D), bf16),
        pltpu.VMEM((S, D), bf16),
        pltpu.VMEM((6, D, NMODE), bf16),
        pltpu.VMEM((D,), bf16),
        pltpu.VMEM((D,), bf16),
        pltpu.VMEM((6, 2 * T, T), bf16),
        pltpu.VMEM((T, 2 * T), bf16),
        pltpu.VMEM((8, 32, 128), u32),
        pltpu.VMEM((D // 2, D), u32),
        pltpu.VMEM((D // 2, 2 * D), u32),
        pltpu.VMEM((D // 2, D), u32),
        pltpu.VMEM((T, T), u32),
        pltpu.VMEM((5, T, T), u32),
        pltpu.VMEM((T // 2, 2 * T), u32),
        pltpu.VMEM((S // 2, D), u32),
        pltpu.VMEM((S // 2, D), u32),
        pltpu.VMEM((D // 2, S), u32),
        pltpu.VMEM((UNR, D, T), f32),
        pltpu.VMEM((4, 256, 128), f32),
        pltpu.VMEM((4, 256, 128), f32),
        pltpu.VMEM((4, D, NMODE), f32),
        pltpu.VMEM((D, NMODE), f32),
        pltpu.VMEM((8, D), f32),
        pltpu.VMEM((4, 8, 80, 128), f32),
        pltpu.VMEM((20, 128, 128), f32),
        pltpu.VMEM((20, 128, 128), f32),
        pltpu.VMEM((4, 768, 128), f32),
        pltpu.VMEM((3, NCH, 4, T, 128), f32),
        pltpu.VMEM((3, NCH, 4, T, 128), f32),
        pltpu.VMEM((NCH + 2, 4, 3 * T, 128), f32),
        pltpu.VMEM((S + 16, D), bf16),
        pltpu.VMEM((S, D), bf16),
        pltpu.SemaphoreType.DMA((16,)),
        pltpu.SemaphoreType.DMA((2 * NCH,)),
        pltpu.SemaphoreType.DMA((2 * NCH,)),
    ]
    call = pl.pallas_call(
        _kernel,
        out_shape=jax.ShapeDtypeStruct((1, S, 2 * D), bf16),
        in_specs=[anyspec] * 15,
        out_specs=anyspec,
        scratch_shapes=scratch,
        compiler_params=pltpu.CompilerParams(vmem_limit_bytes=110 * 1024 * 1024),
    )
    return call(A_x, A_wqkv, A_wo, B_u, B_A_re, B_A_im, B_B_re, B_B_im, B_C_re, B_C_im, B_log_dt, B_Dskip,
                jnp.asarray(DFT_NP), jnp.asarray(G_NP), jnp.asarray(HM_NP))
```
